```python
import jax
import jax.numpy as jnp

def _softmax(x, axis=-1):
    return jax.nn.softmax(x, axis=axis)
def _gelu(x):
    return jax.nn.gelu(x, approximate=True)
def _silu(x):
    return jax.nn.silu(x)
def _sigmoid(x):
    return jax.nn.sigmoid(x)
def _layernorm(x, axis=-1, eps=1e-5):
    m = jnp.mean(x, axis=axis, keepdims=True)
    v = jnp.var(x, axis=axis, keepdims=True)
    return (x - m) / jnp.sqrt(v + eps)
def _scatter_add(tgt, idx, src, axis=0):
    return tgt.at[idx].add(src)
def _segment_sum(src, seg, n):
    return jax.ops.segment_sum(src, seg, n)
class _Rng:
    def __init__(self, key):
        self._k = key
    def _next(self):
        self._k, sub = jax.random.split(self._k)
        return sub
    def normal(self, shape):
        return jax.random.normal(self._next(), shape, dtype=jnp.bfloat16)
    def randint(self, lo, hi, shape):
        return jax.random.randint(self._next(), shape, lo, hi, dtype=jnp.int32)
    def uniform(self, shape, lo=0.0, hi=1.0):
        return jax.random.uniform(self._next(), shape, jnp.bfloat16, lo, hi)
    def permutation(self, n):
        return jax.random.permutation(self._next(), n)


kernel_name = 'gated_mix__mha_block_cached__moe_arch_mod__decode'

def setup_inputs():
    _rng = _Rng(jax.random.key(int.from_bytes(__import__("os").urandom(4), "little")))
    _w = (lambda a: (lambda t: t.astype(jnp.bfloat16) if jnp.issubdtype(t.dtype, jnp.floating) else t)(jnp.asarray(a)))
    def _A_setup():
        B, Sq, D = 4, 1, 1024
        H, Sk, Dh = 32, 8192, 128
        return {
            "x": _w((lambda *s: _rng.normal(s) * 0.05)(B, Sq, D)),
            "k_cache": _w((lambda *s: _rng.normal(s) * 0.05)(B, H, Sk, Dh)),
            "v_cache": _w((lambda *s: _rng.normal(s) * 0.05)(B, H, Sk, Dh)),
            "wq": _w((lambda *s: _rng.normal(s) * 0.05)(D, H * Dh) * (D ** -0.5)),
            "wo": _w((lambda *s: _rng.normal(s) * 0.05)(H * Dh, D) * ((H * Dh) ** -0.5)),
        }
    _A_in = _A_setup()

    def _B_setup():
        B, S, D, F, C = 4, 1, 1024, 3584, 1
        return {
            "x": _w((lambda *s: _rng.normal(s) * 0.05)(B, S, D)),
            "w_r": _w((lambda *s: _rng.normal(s) * 0.05)(D)),
            "w_gate": _w((lambda *s: _rng.normal(s) * 0.05)(D, F)),
            "w_up": _w((lambda *s: _rng.normal(s) * 0.05)(D, F)),
            "w_down": _w((lambda *s: _rng.normal(s) * 0.05)(F, D)),
        }
    _B_in = _B_setup()

    return {
        "A_x": _A_in["x"],
        "A_k_cache": _A_in["k_cache"],
        "A_v_cache": _A_in["v_cache"],
        "A_wq": _A_in["wq"],
        "A_wo": _A_in["wo"],
        "B_x": _B_in["x"],
        "B_w_r": _B_in["w_r"],
        "B_w_gate": _B_in["w_gate"],
        "B_w_up": _B_in["w_up"],
        "B_w_down": _B_in["w_down"],
        "gate_w": _w((lambda *s: _rng.normal(s) * 0.05)(1024)),
    }

def reference(A_x, A_k_cache, A_v_cache, A_wq, A_wo, B_x, B_w_r, B_w_gate, B_w_up, B_w_down, gate_w):
    def _A_ref(x, k_cache, v_cache, wq, wo):
        B, Sq, D = x.shape
        H, Dh = 32, 128
        q = (lambda x, *d: x.transpose(*d))((x @ wq).reshape(B, Sq, H, Dh), 0, 2, 1, 3)
        scores = jnp.einsum("bhqd,bhkd->bhqk", q, k_cache) * (Dh ** -0.5)
        p = _softmax(scores, axis=-1)
        o = jnp.einsum("bhqk,bhkd->bhqd", p, v_cache)
        return (lambda x, *d: x.transpose(*d))(o, 0, 2, 1, 3).reshape(B, Sq, H * Dh) @ wo

    def _B_ref(x, w_r, w_gate, w_up, w_down):
        B, S, D = x.shape
        C = 1
        r = x @ w_r
        idx = jnp.argsort(-r, axis=-1)[:, :C]
        idx_e = jnp.repeat(idx.reshape(B, C, 1), D, axis=2)
        x_sel = jnp.take_along_axis(x, idx_e, axis=1)
        g = _silu(x_sel @ w_gate)
        u = x_sel @ w_up
        y = (g * u) @ w_down
        r_sel = _sigmoid(jnp.take_along_axis(r, idx, axis=1))
        y = y * r_sel.reshape(B, C, 1)
        b_off = (jnp.arange(B) * S).reshape(B, 1)
        flat_idx = (idx + b_off).reshape(B * C)
        zero = (x * 0.0).reshape(B * S, D)
        upd = _scatter_add(zero, flat_idx, y.reshape(B * C, D), axis=0)
        return x + upd.reshape(B, S, D)

    x = A_x
    g = _sigmoid((x * gate_w).sum(-1, keepdims=True))
    a = _A_ref(x, A_k_cache, A_v_cache, A_wq, A_wo)
    b = _B_ref(x, B_w_r, B_w_gate, B_w_up, B_w_down)
    return g * a + (1 - g) * b
```

```python
import functools
import jax
import jax.numpy as jnp
from jax import lax
import jax.experimental.pallas as pl
import jax.experimental.pallas.tpu as pltpu

B, D, H, SK, DH, F = 4, 1024, 32, 8192, 128, 3584


def _kernel(x_hbm, wr_hbm, gw_hbm, k_hbm, v_hbm, wq_hbm, wo_hbm, wg_hbm, wu_hbm, wd_hbm,
            o_ref, x_v, wr_v, gw_v, kbuf, vbuf, wq_v, wo_v, wg_v, wu_v, wd_v, q_s, o_s, sem_k, sem_v, sem_w, sem_o,
            *, nbuf, rows, kb, wo_chunks, early):
    n_pairs = B * H
    nblk = SK // kb
    half = kb // 2
    n = half // rows

    def issue_blk(i, j, slot):
        h = i // B
        b = i % B
        for c in range(n):
            for s in range(2):
                src = pl.ds(pl.multiple_of(s * (SK // 2) + j * half + c * rows, rows), rows)
                dst = pl.ds(s * half + c * rows, rows)
                pltpu.make_async_copy(k_hbm.at[b, h, src], kbuf.at[slot, dst], sem_k.at[slot]).start(priority=0)
                pltpu.make_async_copy(v_hbm.at[b, h, src], vbuf.at[slot, dst], sem_v.at[slot]).start(priority=1)

    def issue_w(src, dst, sem, r0, nrows, cw):
        ncol = src.shape[1] // cw
        qr = nrows // 4
        def body(t, _):
            for c in range(ncol):
                for s in range(4):
                    r = pl.multiple_of(r0 + s * qr + t * 16, 16)
                    sl = (pl.ds(r, 16), pl.ds(c * cw, cw))
                    pltpu.make_async_copy(src.at[sl], dst.at[sl], sem).start(priority=s % 2)
            return None
        lax.fori_loop(0, qr // 16, body, None)

    c_x = pltpu.make_async_copy(x_hbm, x_v, sem_w.at[0])
    c_wr = pltpu.make_async_copy(wr_hbm, wr_v, sem_w.at[1])
    c_gw = pltpu.make_async_copy(gw_hbm, gw_v, sem_w.at[2])
    c_x.start()
    c_wr.start()
    c_gw.start()
    issue_w(wq_hbm, wq_v, sem_w.at[3], 0, D, 1024)
    issue_w(wg_hbm, wg_v, sem_w.at[4], 0, D, 896)

    c_x.wait()
    c_wr.wait()
    c_gw.wait()
    x = x_v[...]
    xf = x.astype(jnp.float32)
    wr = wr_v[...].astype(jnp.float32)
    gw = gw_v[...].astype(jnp.float32)
    gsum = jnp.zeros((B, 128), jnp.float32)
    rsum = jnp.zeros((B, 128), jnp.float32)
    for c in range(D // 128):
        xc = xf[:, c * 128:(c + 1) * 128]
        gsum = gsum + xc * gw[c:c + 1, :]
        rsum = rsum + xc * wr[c:c + 1, :]
    gate = jax.nn.sigmoid(jnp.sum(gsum, axis=-1, keepdims=True))
    r_sel = jax.nn.sigmoid(jnp.sum(rsum, axis=-1, keepdims=True))

    def wait_all(buf, sem):
        pltpu.make_async_copy(buf, buf, sem).wait()

    wait_all(wq_v, sem_w.at[3])
    q_s[...] = jnp.dot(x, wq_v[...], preferred_element_type=jnp.float32)
    issue_w(wu_hbm, wu_v, sem_w.at[5], 0, D, 896)
    wait_all(wg_v, sem_w.at[4])
    g = jnp.dot(x, wg_v[...], preferred_element_type=jnp.float32)
    g = g * jax.nn.sigmoid(g)
    issue_w(wd_hbm, wd_v, sem_w.at[6], 0, F, 1024)
    wait_all(wu_v, sem_w.at[5])
    u = jnp.dot(x, wu_v[...], preferred_element_type=jnp.float32)
    hid = (g * u).astype(jnp.bfloat16)
    for s in range(nbuf):
        issue_blk(s // nblk, s % nblk, s)
    wait_all(wd_v, sem_w.at[6])
    y = jnp.dot(hid, wd_v[...], preferred_element_type=jnp.float32)
    y = y * r_sel
    bres = xf + (xf * 0.0 + y)

    row4 = lax.broadcasted_iota(jnp.int32, (B, DH), 0)
    wo_rows = H * DH // wo_chunks
    o_s[...] = jnp.zeros_like(o_s)

    def pair_body(i, _):
        h = i // B
        b = i % B
        hs = pl.multiple_of(h * DH, DH)
        qh = q_s[:, pl.ds(hs, DH)]
        qrow = jnp.sum(jnp.where(row4 == b, qh, 0.0), axis=0, keepdims=True)
        qb = jnp.broadcast_to(qrow, (8, DH)).astype(jnp.bfloat16)
        m = l = acc = None
        for j in range(nblk):
            t = i * nblk + j
            slot = t % nbuf if nblk % nbuf else j % nbuf
            wait_all(kbuf.at[slot], sem_k.at[slot])
            s = lax.dot_general(qb, kbuf[slot], (((1,), (1,)), ((), ())), preferred_element_type=jnp.float32)
            s = s * (DH ** -0.5)
            mb = jnp.max(s, axis=-1, keepdims=True)
            m_new = mb if j == 0 else jnp.maximum(m, mb)
            p = jnp.exp(s - m_new)
            lb = jnp.sum(p, axis=-1, keepdims=True)
            wait_all(vbuf.at[slot], sem_v.at[slot])
            pv = jnp.dot(p.astype(jnp.bfloat16), vbuf[slot], preferred_element_type=jnp.float32)
            if j == 0:
                l, acc = lb, pv
            else:
                alpha = jnp.exp(m - m_new)
                l = alpha * l + lb
                acc = alpha * acc + pv
            m = m_new
            jn = (j + nbuf) % nblk
            inx = i + (j + nbuf) // nblk

            @pl.when(inx < n_pairs)
            def _():
                issue_blk(inx, jn, slot)

            tt = t + nbuf - n_pairs * nblk
            @pl.when(jnp.logical_and(tt >= 0, tt < early))
            def _():
                issue_w(wo_hbm, wo_v, sem_o.at[tt], tt * wo_rows, wo_rows, 1024)
        o_row = (acc / l)[0:B]
        o_s[:, pl.ds(hs, DH)] = jnp.where(row4 == b, o_row, o_s[:, pl.ds(hs, DH)])
        return None

    lax.fori_loop(0, n_pairs, pair_body, None)
    a = jnp.zeros((B, D), jnp.float32)
    for c in range(wo_chunks):
        sl = pl.ds(c * wo_rows, wo_rows)
        wait_all(wo_v.at[sl], sem_o.at[c])
        if c + early < wo_chunks:
            issue_w(wo_hbm, wo_v, sem_o.at[c + early], (c + early) * wo_rows, wo_rows, 1024)
        a = a + jnp.dot(o_s[:, sl].astype(jnp.bfloat16), wo_v[sl, :], preferred_element_type=jnp.float32)
    o_ref[...] = (gate * a + (1.0 - gate) * bres).astype(o_ref.dtype)


def _make(nbuf=4, rows=128, kb=2048, wo_chunks=8, early=None):
    early = min(nbuf, wo_chunks) if early is None else early
    assert early <= nbuf
    @jax.jit
    def f(A_x, A_k_cache, A_v_cache, A_wq, A_wo, B_x, B_w_r, B_w_gate, B_w_up, B_w_down, gate_w):
        any_spec = pl.BlockSpec(memory_space=pl.ANY)
        vm = pl.BlockSpec(memory_space=pltpu.VMEM)
        out = pl.pallas_call(
            functools.partial(_kernel, nbuf=nbuf, rows=rows, kb=kb, wo_chunks=wo_chunks, early=early),
            in_specs=[any_spec] * 10,
            out_specs=vm,
            out_shape=jax.ShapeDtypeStruct((B, D), A_x.dtype),
            scratch_shapes=[
                pltpu.VMEM((B, D), jnp.bfloat16),
                pltpu.VMEM((8, 128), jnp.bfloat16),
                pltpu.VMEM((8, 128), jnp.bfloat16),
                pltpu.VMEM((nbuf, kb, DH), jnp.bfloat16),
                pltpu.VMEM((nbuf, kb, DH), jnp.bfloat16),
                pltpu.VMEM((D, H * DH), jnp.bfloat16),
                pltpu.VMEM((H * DH, D), jnp.bfloat16),
                pltpu.VMEM((D, F), jnp.bfloat16),
                pltpu.VMEM((D, F), jnp.bfloat16),
                pltpu.VMEM((F, D), jnp.bfloat16),
                pltpu.VMEM((B, H * DH), jnp.float32),
                pltpu.VMEM((B, H * DH), jnp.float32),
                pltpu.SemaphoreType.DMA((nbuf,)),
                pltpu.SemaphoreType.DMA((nbuf,)),
                pltpu.SemaphoreType.DMA((7,)),
                pltpu.SemaphoreType.DMA((wo_chunks,)),
            ],
            compiler_params=pltpu.CompilerParams(vmem_limit_bytes=120 * 1024 * 1024),
        )(A_x.reshape(B, D), B_w_r.reshape(8, 128), gate_w.reshape(8, 128),
          A_k_cache, A_v_cache, A_wq, A_wo, B_w_gate, B_w_up, B_w_down)
        return out.reshape(B, 1, D)
    return f


_impl = _make(nbuf=4, rows=128, kb=2048)


@jax.jit
def pallas_gated_mix__mha_block_cached__moe_arch_mod__decode_kernel(
    A_x, A_k_cache, A_v_cache, A_wq, A_wo, B_x, B_w_r, B_w_gate, B_w_up, B_w_down, gate_w
):
    return _impl(A_x, A_k_cache, A_v_cache, A_wq, A_wo, B_x, B_w_r, B_w_gate, B_w_up, B_w_down, gate_w)
```

```python
import jax
import jax.numpy as jnp
from jax import lax
import jax.experimental.pallas as pl
import jax.experimental.pallas.tpu as pltpu

B, D, H, SK, DH, F = 4, 1024, 32, 8192, 128, 3584
KB = 2048
NBLK = SK // KB
N_STREAMS = 3
N_PIECES = 4
WO_CHUNKS = 8
WO_ROWS = H * DH // WO_CHUNKS
assert NBLK <= WO_CHUNKS


def _split(total, n, rot=0):
    base, rem = divmod(total, n)
    return [base + ((i + rot + 1) * rem) // n - ((i + rot) * rem) // n for i in range(n)]


def _block_plan():
    lens = _split(KB // 16, N_STREAMS)
    plan = []
    for p in range(N_PIECES):
        for s in range(N_STREAMS):
            sizes = _split(lens[s], N_PIECES, s)
            off = 16 * sum(sizes[:p])
            before = 16 * sum(lens[:s])
            plan.append((before * NBLK + off, 16 * lens[s], before + off, 16 * sizes[p]))
    return plan


def _kernel(x_hbm, wr_hbm, gw_hbm, k_hbm, v_hbm, wq_hbm, wo_hbm, wg_hbm, wu_hbm, wd_hbm,
            o_ref,
            x_v, wr_v, gw_v, kbuf, vbuf, wq_v, wo_v, wg_v, wu_v, wd_v, q_s, o_s,
            sem_k, sem_v, sem_w, sem_o):
    n_pairs = B * H
    plan = _block_plan()

    def issue_block(i, j):
        h = i // B
        b = i % B
        for (src0, step, dst0, nr) in plan:
            src = pl.ds(src0 + j * step, nr)
            dst = pl.ds(dst0, nr)
            pltpu.make_async_copy(k_hbm.at[b, h, src], kbuf.at[j, dst], sem_k.at[j]).start(priority=0)
            pltpu.make_async_copy(v_hbm.at[b, h, src], vbuf.at[j, dst], sem_v.at[j]).start(priority=1)

    def issue_weight(src, dst, sem, r0, nrows, cw):
        qr = nrows // 4

        def body(t, _):
            for c in range(src.shape[1] // cw):
                for s in range(4):
                    r = pl.multiple_of(r0 + s * qr + t * 16, 16)
                    sl = (pl.ds(r, 16), pl.ds(c * cw, cw))
                    pltpu.make_async_copy(src.at[sl], dst.at[sl], sem).start(priority=s % 2)

        lax.fori_loop(0, qr // 16, body, None)

    def wait_all(buf, sem):
        pltpu.make_async_copy(buf, buf, sem).wait()

    c_x = pltpu.make_async_copy(x_hbm, x_v, sem_w.at[0])
    c_wr = pltpu.make_async_copy(wr_hbm, wr_v, sem_w.at[1])
    c_gw = pltpu.make_async_copy(gw_hbm, gw_v, sem_w.at[2])
    c_x.start()
    c_wr.start()
    c_gw.start()
    issue_weight(wq_hbm, wq_v, sem_w.at[3], 0, D, 1024)
    issue_weight(wg_hbm, wg_v, sem_w.at[4], 0, D, 896)

    c_x.wait()
    c_wr.wait()
    c_gw.wait()
    x = x_v[...]
    xf = x.astype(jnp.float32)
    wr = wr_v[...].astype(jnp.float32)
    gw = gw_v[...].astype(jnp.float32)
    gsum = jnp.zeros((B, 128), jnp.float32)
    rsum = jnp.zeros((B, 128), jnp.float32)
    for c in range(D // 128):
        xc = xf[:, c * 128:(c + 1) * 128]
        gsum = gsum + xc * gw[c:c + 1, :]
        rsum = rsum + xc * wr[c:c + 1, :]
    gate = jax.nn.sigmoid(jnp.sum(gsum, axis=-1, keepdims=True))
    r_sel = jax.nn.sigmoid(jnp.sum(rsum, axis=-1, keepdims=True))

    wait_all(wq_v, sem_w.at[3])
    q_s[...] = jnp.dot(x, wq_v[...], preferred_element_type=jnp.float32)
    issue_weight(wu_hbm, wu_v, sem_w.at[5], 0, D, 896)
    wait_all(wg_v, sem_w.at[4])
    g = jnp.dot(x, wg_v[...], preferred_element_type=jnp.float32)
    g = g * jax.nn.sigmoid(g)
    issue_weight(wd_hbm, wd_v, sem_w.at[6], 0, F, 1024)
    wait_all(wu_v, sem_w.at[5])
    u = jnp.dot(x, wu_v[...], preferred_element_type=jnp.float32)
    hid = (g * u).astype(jnp.bfloat16)
    for j in range(NBLK):
        issue_block(0, j)
    wait_all(wd_v, sem_w.at[6])
    y = jnp.dot(hid, wd_v[...], preferred_element_type=jnp.float32) * r_sel
    b_out = xf + (xf * 0.0 + y)

    row = lax.broadcasted_iota(jnp.int32, (B, DH), 0)
    o_s[...] = jnp.zeros_like(o_s)

    def pair_body(i, _):
        h = i // B
        b = i % B
        cols = pl.ds(pl.multiple_of(h * DH, DH), DH)
        q_row = jnp.sum(jnp.where(row == b, q_s[:, cols], 0.0), axis=0, keepdims=True)
        q = jnp.broadcast_to(q_row, (8, DH)).astype(jnp.bfloat16)
        m = l = acc = None
        for j in range(NBLK):
            wait_all(kbuf.at[j], sem_k.at[j])
            s = lax.dot_general(q, kbuf[j], (((1,), (1,)), ((), ())),
                                preferred_element_type=jnp.float32) * (DH ** -0.5)
            m_blk = jnp.max(s, axis=-1, keepdims=True)
            m_new = m_blk if j == 0 else jnp.maximum(m, m_blk)
            p = jnp.exp(s - m_new)
            l_blk = jnp.sum(p, axis=-1, keepdims=True)
            wait_all(vbuf.at[j], sem_v.at[j])
            pv = jnp.dot(p.astype(jnp.bfloat16), vbuf[j], preferred_element_type=jnp.float32)
            if j == 0:
                l, acc = l_blk, pv
            else:
                alpha = jnp.exp(m - m_new)
                l = alpha * l + l_blk
                acc = alpha * acc + pv
            m = m_new

            @pl.when(i + 1 < n_pairs)
            def _():
                issue_block(i + 1, j)

            @pl.when(i + 1 == n_pairs)
            def _():
                issue_weight(wo_hbm, wo_v, sem_o.at[j], j * WO_ROWS, WO_ROWS, 1024)

        o_s[:, cols] = jnp.where(row == b, (acc / l)[0:B], o_s[:, cols])

    lax.fori_loop(0, n_pairs, pair_body, None)

    a = jnp.zeros((B, D), jnp.float32)
    for c in range(WO_CHUNKS):
        rows = pl.ds(c * WO_ROWS, WO_ROWS)
        wait_all(wo_v.at[rows], sem_o.at[c])
        if c + NBLK < WO_CHUNKS:
            issue_weight(wo_hbm, wo_v, sem_o.at[c + NBLK], (c + NBLK) * WO_ROWS, WO_ROWS, 1024)
        a = a + jnp.dot(o_s[:, rows].astype(jnp.bfloat16), wo_v[rows, :],
                        preferred_element_type=jnp.float32)
    o_ref[...] = (gate * a + (1.0 - gate) * b_out).astype(o_ref.dtype)


@jax.jit
def pallas_gated_mix__mha_block_cached__moe_arch_mod__decode_kernel(
    A_x: jax.Array,
    A_k_cache: jax.Array,
    A_v_cache: jax.Array,
    A_wq: jax.Array,
    A_wo: jax.Array,
    B_x: jax.Array,
    B_w_r: jax.Array,
    B_w_gate: jax.Array,
    B_w_up: jax.Array,
    B_w_down: jax.Array,
    gate_w: jax.Array,
):
    del B_x
    bf16 = jnp.bfloat16
    out = pl.pallas_call(
        _kernel,
        in_specs=[pl.BlockSpec(memory_space=pl.ANY)] * 10,
        out_specs=pl.BlockSpec(memory_space=pltpu.VMEM),
        out_shape=jax.ShapeDtypeStruct((B, D), A_x.dtype),
        scratch_shapes=[
            pltpu.VMEM((B, D), bf16),
            pltpu.VMEM((8, 128), bf16),
            pltpu.VMEM((8, 128), bf16),
            pltpu.VMEM((NBLK, KB, DH), bf16),
            pltpu.VMEM((NBLK, KB, DH), bf16),
            pltpu.VMEM((D, H * DH), bf16),
            pltpu.VMEM((H * DH, D), bf16),
            pltpu.VMEM((D, F), bf16),
            pltpu.VMEM((D, F), bf16),
            pltpu.VMEM((F, D), bf16),
            pltpu.VMEM((B, H * DH), jnp.float32),
            pltpu.VMEM((B, H * DH), jnp.float32),
            pltpu.SemaphoreType.DMA((NBLK,)),
            pltpu.SemaphoreType.DMA((NBLK,)),
            pltpu.SemaphoreType.DMA((7,)),
            pltpu.SemaphoreType.DMA((WO_CHUNKS,)),
        ],
        compiler_params=pltpu.CompilerParams(vmem_limit_bytes=100 * 1024 * 1024),
    )(A_x.reshape(B, D), B_w_r.reshape(8, 128), gate_w.reshape(8, 128),
      A_k_cache, A_v_cache, A_wq, A_wo, B_w_gate, B_w_up, B_w_down)
    return out.reshape(B, 1, D)
```

```python
import jax
import jax.numpy as jnp
from jax import lax
import jax.experimental.pallas as pl
import jax.experimental.pallas.tpu as pltpu

B, D, H, SK, DH, F = 4, 1024, 32, 8192, 128, 3584
KB = 2048
NBLK = SK // KB
STREAMS = (43, 42, 43)
N_PIECES = 4
WO_CHUNKS = 8
WO_ROWS = H * DH // WO_CHUNKS
assert NBLK <= WO_CHUNKS


def _split(total, n, rot=0):
    base, rem = divmod(total, n)
    return [base + ((i + rot + 1) * rem) // n - ((i + rot) * rem) // n for i in range(n)]


def _block_plan():
    lens = STREAMS
    assert 16 * sum(lens) == KB
    plan = []
    for p in range(N_PIECES):
        for s in range(len(lens)):
            sizes = _split(lens[s], N_PIECES, s)
            off = 16 * sum(sizes[:p])
            before = 16 * sum(lens[:s])
            plan.append((before * NBLK + off, 16 * lens[s], before + off, 16 * sizes[p]))
    return plan


def _kernel(x_hbm, wr_hbm, gw_hbm, k_hbm, v_hbm, wq_hbm, wo_hbm, wg_hbm, wu_hbm, wd_hbm,
            o_ref,
            x_v, wr_v, gw_v, kbuf, vbuf, wq_v, wo_v, wg_v, wu_v, wd_v, q_s, o_s,
            sem_k, sem_v, sem_w, sem_o):
    n_pairs = B * H
    plan = _block_plan()

    def issue_block(i, j):
        h = i // B
        b = i % B
        for (src0, step, dst0, nr) in plan:
            src = pl.ds(src0 + j * step, nr)
            dst = pl.ds(dst0, nr)
            pltpu.make_async_copy(k_hbm.at[b, h, src], kbuf.at[j, dst], sem_k.at[j]).start(priority=0)
            pltpu.make_async_copy(v_hbm.at[b, h, src], vbuf.at[j, dst], sem_v.at[j]).start(priority=1)

    def issue_weight(src, dst, sem, r0, nrows, cw):
        qr = nrows // 4

        def body(t, _):
            for c in range(src.shape[1] // cw):
                for s in range(4):
                    r = pl.multiple_of(r0 + s * qr + t * 16, 16)
                    sl = (pl.ds(r, 16), pl.ds(c * cw, cw))
                    pltpu.make_async_copy(src.at[sl], dst.at[sl], sem).start(priority=s % 2)

        lax.fori_loop(0, qr // 16, body, None)

    def wait_all(buf, sem):
        pltpu.make_async_copy(buf, buf, sem).wait()

    c_x = pltpu.make_async_copy(x_hbm, x_v, sem_w.at[0])
    c_wr = pltpu.make_async_copy(wr_hbm, wr_v, sem_w.at[1])
    c_gw = pltpu.make_async_copy(gw_hbm, gw_v, sem_w.at[2])
    c_x.start()
    c_wr.start()
    c_gw.start()
    issue_weight(wq_hbm, wq_v, sem_w.at[3], 0, D, 1024)
    issue_weight(wg_hbm, wg_v, sem_w.at[4], 0, D, 896)

    c_x.wait()
    c_wr.wait()
    c_gw.wait()
    x = x_v[...]
    xf = x.astype(jnp.float32)
    wr = wr_v[...].astype(jnp.float32)
    gw = gw_v[...].astype(jnp.float32)
    gsum = jnp.zeros((B, 128), jnp.float32)
    rsum = jnp.zeros((B, 128), jnp.float32)
    for c in range(D // 128):
        xc = xf[:, c * 128:(c + 1) * 128]
        gsum = gsum + xc * gw[c:c + 1, :]
        rsum = rsum + xc * wr[c:c + 1, :]
    gate = jax.nn.sigmoid(jnp.sum(gsum, axis=-1, keepdims=True))
    r_sel = jax.nn.sigmoid(jnp.sum(rsum, axis=-1, keepdims=True))

    wait_all(wq_v, sem_w.at[3])
    q_s[...] = jnp.dot(x, wq_v[...], preferred_element_type=jnp.float32)
    issue_weight(wu_hbm, wu_v, sem_w.at[5], 0, D, 896)
    wait_all(wg_v, sem_w.at[4])
    g = jnp.dot(x, wg_v[...], preferred_element_type=jnp.float32)
    g = g * jax.nn.sigmoid(g)
    issue_weight(wd_hbm, wd_v, sem_w.at[6], 0, F, 1024)
    wait_all(wu_v, sem_w.at[5])
    u = jnp.dot(x, wu_v[...], preferred_element_type=jnp.float32)
    hid = (g * u).astype(jnp.bfloat16)
    for j in range(NBLK):
        issue_block(0, j)
    wait_all(wd_v, sem_w.at[6])
    y = jnp.dot(hid, wd_v[...], preferred_element_type=jnp.float32) * r_sel
    b_out = xf + (xf * 0.0 + y)

    row = lax.broadcasted_iota(jnp.int32, (B, DH), 0)
    o_s[...] = jnp.zeros_like(o_s)

    def pair_body(i, _):
        h = i // B
        b = i % B
        cols = pl.ds(pl.multiple_of(h * DH, DH), DH)
        q_row = jnp.sum(jnp.where(row == b, q_s[:, cols], 0.0), axis=0, keepdims=True)
        q = jnp.broadcast_to(q_row, (8, DH)).astype(jnp.bfloat16)
        m = l = acc = None
        for j in range(NBLK):
            wait_all(kbuf.at[j], sem_k.at[j])
            s = lax.dot_general(q, kbuf[j], (((1,), (1,)), ((), ())),
                                preferred_element_type=jnp.float32) * (DH ** -0.5)
            m_blk = jnp.max(s, axis=-1, keepdims=True)
            m_new = m_blk if j == 0 else jnp.maximum(m, m_blk)
            p = jnp.exp(s - m_new)
            l_blk = jnp.sum(p, axis=-1, keepdims=True)
            wait_all(vbuf.at[j], sem_v.at[j])
            pv = jnp.dot(p.astype(jnp.bfloat16), vbuf[j], preferred_element_type=jnp.float32)
            if j == 0:
                l, acc = l_blk, pv
            else:
                alpha = jnp.exp(m - m_new)
                l = alpha * l + l_blk
                acc = alpha * acc + pv
            m = m_new

            @pl.when(i + 1 < n_pairs)
            def _():
                issue_block(i + 1, j)

            @pl.when(i + 1 == n_pairs)
            def _():
                issue_weight(wo_hbm, wo_v, sem_o.at[j], j * WO_ROWS, WO_ROWS, 1024)

        o_s[:, cols] = jnp.where(row == b, (acc / l)[0:B], o_s[:, cols])

    lax.fori_loop(0, n_pairs, pair_body, None)

    a = jnp.zeros((B, D), jnp.float32)
    for c in range(WO_CHUNKS):
        rows = pl.ds(c * WO_ROWS, WO_ROWS)
        wait_all(wo_v.at[rows], sem_o.at[c])
        if c + NBLK < WO_CHUNKS:
            issue_weight(wo_hbm, wo_v, sem_o.at[c + NBLK], (c + NBLK) * WO_ROWS, WO_ROWS, 1024)
        a = a + jnp.dot(o_s[:, rows].astype(jnp.bfloat16), wo_v[rows, :],
                        preferred_element_type=jnp.float32)
    o_ref[...] = (gate * a + (1.0 - gate) * b_out).astype(o_ref.dtype)


@jax.jit
def pallas_gated_mix__mha_block_cached__moe_arch_mod__decode_kernel(
    A_x: jax.Array,
    A_k_cache: jax.Array,
    A_v_cache: jax.Array,
    A_wq: jax.Array,
    A_wo: jax.Array,
    B_x: jax.Array,
    B_w_r: jax.Array,
    B_w_gate: jax.Array,
    B_w_up: jax.Array,
    B_w_down: jax.Array,
    gate_w: jax.Array,
):
    del B_x
    bf16 = jnp.bfloat16
    out = pl.pallas_call(
        _kernel,
        in_specs=[pl.BlockSpec(memory_space=pl.ANY)] * 10,
        out_specs=pl.BlockSpec(memory_space=pltpu.VMEM),
        out_shape=jax.ShapeDtypeStruct((B, D), A_x.dtype),
        scratch_shapes=[
            pltpu.VMEM((B, D), bf16),
            pltpu.VMEM((8, 128), bf16),
            pltpu.VMEM((8, 128), bf16),
            pltpu.VMEM((NBLK, KB, DH), bf16),
            pltpu.VMEM((NBLK, KB, DH), bf16),
            pltpu.VMEM((D, H * DH), bf16),
            pltpu.VMEM((H * DH, D), bf16),
            pltpu.VMEM((D, F), bf16),
            pltpu.VMEM((D, F), bf16),
            pltpu.VMEM((F, D), bf16),
            pltpu.VMEM((B, H * DH), jnp.float32),
            pltpu.VMEM((B, H * DH), jnp.float32),
            pltpu.SemaphoreType.DMA((NBLK,)),
            pltpu.SemaphoreType.DMA((NBLK,)),
            pltpu.SemaphoreType.DMA((7,)),
            pltpu.SemaphoreType.DMA((WO_CHUNKS,)),
        ],
        compiler_params=pltpu.CompilerParams(vmem_limit_bytes=100 * 1024 * 1024),
    )(A_x.reshape(B, D), B_w_r.reshape(8, 128), gate_w.reshape(8, 128),
      A_k_cache, A_v_cache, A_wq, A_wo, B_w_gate, B_w_up, B_w_down)
    return out.reshape(B, 1, D)
```
